```python
import jax
import jax.numpy as jnp

def _softmax(x, axis=-1):
    return jax.nn.softmax(x, axis=axis)
def _gelu(x):
    return jax.nn.gelu(x, approximate=True)
def _silu(x):
    return jax.nn.silu(x)
def _sigmoid(x):
    return jax.nn.sigmoid(x)
def _layernorm(x, axis=-1, eps=1e-5):
    m = jnp.mean(x, axis=axis, keepdims=True)
    v = jnp.var(x, axis=axis, keepdims=True)
    return (x - m) / jnp.sqrt(v + eps)
def _scatter_add(tgt, idx, src, axis=0):
    return tgt.at[idx].add(src)
def _segment_sum(src, seg, n):
    return jax.ops.segment_sum(src, seg, n)
class _Rng:
    def __init__(self, key):
        self._k = key
    def _next(self):
        self._k, sub = jax.random.split(self._k)
        return sub
    def normal(self, shape):
        return jax.random.normal(self._next(), shape, dtype=jnp.bfloat16)
    def randint(self, lo, hi, shape):
        return jax.random.randint(self._next(), shape, lo, hi, dtype=jnp.int32)
    def uniform(self, shape, lo=0.0, hi=1.0):
        return jax.random.uniform(self._next(), shape, jnp.bfloat16, lo, hi)
    def permutation(self, n):
        return jax.random.permutation(self._next(), n)


kernel_name = 'concat_heads__compressed_kv_cla__gqa_block_cached__decode'

def setup_inputs():
    _rng = _Rng(jax.random.key(int.from_bytes(__import__("os").urandom(4), "little")))
    _w = (lambda a: (lambda t: t.astype(jnp.bfloat16) if jnp.issubdtype(t.dtype, jnp.floating) else t)(jnp.asarray(a)))
    def _A_setup():
        B, H, Sq, Sk, D, M = 2, 32, 1, 4096, 128, 512
        Dc = 4 * D
        return {
            "x": _w((lambda *s: _rng.normal(s) * 0.05)(B, Sq, M)),
            "c_kv": _w((lambda *s: _rng.normal(s) * 0.05)(B, Sk, Dc)),
            "w_q": _w((lambda *s: _rng.normal(s) * 0.05)(M, H, D) * (M ** -0.5)),
            "w_uk": _w((lambda *s: _rng.normal(s) * 0.05)(Dc, H, D) * (Dc ** -0.5)),
            "w_uv": _w((lambda *s: _rng.normal(s) * 0.05)(Dc, H, D) * (Dc ** -0.5)),
            "w_o": _w((lambda *s: _rng.normal(s) * 0.05)(H, D, M) * ((H * D) ** -0.5)),
        }
    _A_in = _A_setup()

    def _B_setup():
        B, Sq, D = 2, 1, 512
        Hq, Hkv, Sk, Dh = 32, 32, 4096, 128
        assert Hq % Hkv == 0, (Hq, Hkv)
        return {
            "x": _w((lambda *s: _rng.normal(s) * 0.05)(B, Sq, D)),
            "k_cache": _w((lambda *s: _rng.normal(s) * 0.05)(B, Hkv, Sk, Dh)),
            "v_cache": _w((lambda *s: _rng.normal(s) * 0.05)(B, Hkv, Sk, Dh)),
            "wq": _w((lambda *s: _rng.normal(s) * 0.05)(D, Hq * Dh) * (D ** -0.5)),
            "wo": _w((lambda *s: _rng.normal(s) * 0.05)(Hq * Dh, D) * ((Hq * Dh) ** -0.5)),
        }
    _B_in = _B_setup()

    return {
        "A_x": _A_in["x"],
        "A_c_kv": _A_in["c_kv"],
        "A_w_q": _A_in["w_q"],
        "A_w_uk": _A_in["w_uk"],
        "A_w_uv": _A_in["w_uv"],
        "A_w_o": _A_in["w_o"],
        "B_x": _B_in["x"],
        "B_k_cache": _B_in["k_cache"],
        "B_v_cache": _B_in["v_cache"],
        "B_wq": _B_in["wq"],
        "B_wo": _B_in["wo"],
    }

def reference(A_x, A_c_kv, A_w_q, A_w_uk, A_w_uv, A_w_o, B_x, B_k_cache, B_v_cache, B_wq, B_wo):
    def _A_ref(x, c_kv, w_q, w_uk, w_uv, w_o):
        B, Sq, M = x.shape[0], x.shape[1], x.shape[2]
        Sk = c_kv.shape[1]
        H, D = w_q.shape[1], w_q.shape[2]
        q = jnp.einsum("bqm,mhd->bhqd", x, w_q)
        k = jnp.einsum("bkc,chd->bhkd", c_kv, w_uk)
        v = jnp.einsum("bkc,chd->bhkd", c_kv, w_uv)
        scores = jnp.einsum("bhqd,bhkd->bhqk", q, k) * (D ** -0.5)
        off = Sk - Sq
        qi = jnp.arange(Sq)[:, None]
        kj = jnp.arange(Sk)[None, :]
        cmask = kj <= (qi + off)
        scores = jnp.where(cmask[None, None], scores, -1e9)
        p = _softmax(scores, axis=-1)
        ctx = jnp.einsum("bhqk,bhkd->bhqd", p, v)
        return jnp.einsum("bhqd,hdm->bqm", ctx, w_o)

    def _B_ref(x, k_cache, v_cache, wq, wo):
        B, Sq, D = x.shape
        Hq, Dh = 32, 128
        Hkv = k_cache.shape[1]
        rep = Hq // Hkv
        q = (lambda x, *d: x.transpose(*d))((x @ wq).reshape(B, Sq, Hq, Dh), 0, 2, 1, 3)
        k = jnp.repeat(k_cache, rep, axis=1)
        v = jnp.repeat(v_cache, rep, axis=1)
        scores = jnp.einsum("bhqd,bhkd->bhqk", q, k) * (Dh ** -0.5)
        p = _softmax(scores, axis=-1)
        o = jnp.einsum("bhqk,bhkd->bhqd", p, v)
        return (lambda x, *d: x.transpose(*d))(o, 0, 2, 1, 3).reshape(B, Sq, Hq * Dh) @ wo

    a = _A_ref(A_x, A_c_kv, A_w_q, A_w_uk, A_w_uv, A_w_o)
    b = _B_ref(B_x, B_k_cache, B_v_cache, B_wq, B_wo)
    return jnp.concatenate([a, b], axis=-1)
```

```python
import jax
import jax.numpy as jnp
import jax.experimental.pallas as pl
import jax.experimental.pallas.tpu as pltpu

_NBUF = 8
_WO_CHUNKS = 8

_NT = (((1,), (1,)), ((), ()))
_NN = (((1,), (0,)), ((), ()))


def _dot(a, b, dims=_NN):
    return jax.lax.dot_general(a, b, dims, preferred_element_type=jnp.float32)


def _rows_per_batch(x_ref):
    n = x_ref.shape[-1]
    rows = [
        jnp.broadcast_to(x_ref[b].astype(jnp.float32), (8, n)) for b in range(2)
    ]
    return jnp.concatenate(rows, axis=0).astype(jnp.bfloat16)


def _head_pair(w32_ref, j, n_rows, n_pairs):
    w = w32_ref[pl.ds(j, n_rows, stride=n_pairs), :]
    lo = pltpu.bitcast(w << 16, jnp.float32)
    hi = pltpu.bitcast(w & jnp.uint32(0xFFFF0000), jnp.float32)
    return lo.astype(jnp.bfloat16), hi.astype(jnp.bfloat16)


def _kernel(
    xa_hbm, ckv_hbm, wqa_hbm, wuk_hbm, wuv_hbm, woa_hbm,
    xb_hbm, k_hbm, v_hbm, wqb_hbm, wob_hbm,
    out_ref,
    xa_v, xb_v, ckv_v, wqa_v, wuk_v, wuv_v, woa_v, wqb_v, wob_v,
    k_v, v_v, qb_v, ctxa_v, ctxb_v,
    w_sem, wo_sem, k_sem, v_sem,
):
    n_batch, n_heads, _, d_head = k_hbm.shape
    d_model = xa_hbm.shape[-1]
    d_lat = ckv_hbm.shape[-1]
    n_pairs = n_heads // 2
    n_steps = n_batch * n_heads
    scale = d_head ** -0.5
    heads_per_chunk = n_heads // _WO_CHUNKS
    rows_per_chunk = heads_per_chunk * d_head

    cp_xb = pltpu.make_async_copy(xb_hbm, xb_v, w_sem.at[0])
    cp_xa = pltpu.make_async_copy(xa_hbm, xa_v, w_sem.at[1])
    cp_wqb = pltpu.make_async_copy(wqb_hbm, wqb_v, w_sem.at[2])
    cp_wqa = pltpu.make_async_copy(wqa_hbm, wqa_v, w_sem.at[3])
    cp_wuk = pltpu.make_async_copy(wuk_hbm, wuk_v, w_sem.at[4])
    cp_ckv = [
        pltpu.make_async_copy(ckv_hbm.at[b], ckv_v.at[b], w_sem.at[5 + b])
        for b in range(n_batch)
    ]
    cp_wuv = pltpu.make_async_copy(wuv_hbm, wuv_v, w_sem.at[5 + n_batch])

    def cp_wo(which, c):
        src, dst = ((woa_hbm, woa_v), (wob_hbm, wob_v))[which]
        rows = pl.ds(c * rows_per_chunk, rows_per_chunk)
        return pltpu.make_async_copy(
            src.at[rows], dst.at[rows], wo_sem.at[which * _WO_CHUNKS + c]
        )

    def cp_k(step, slot):
        return pltpu.make_async_copy(
            k_hbm.at[step // n_heads, step % n_heads], k_v.at[slot], k_sem.at[slot]
        )

    def cp_v(step, slot):
        return pltpu.make_async_copy(
            v_hbm.at[step // n_heads, step % n_heads], v_v.at[slot], v_sem.at[slot]
        )

    for cp in (cp_xb, cp_xa, cp_wqb, cp_wqa, cp_wuk, *cp_ckv, cp_wuv):
        cp.start()
    for s in range(_NBUF):
        cp_k(s, s).start()
        cp_v(s, s).start()

    cp_xb.wait()
    cp_wqb.wait()
    xb = _rows_per_batch(xb_v)
    for h in range(0, n_heads, 4):
        q4 = _dot(xb, wqb_v[:, h * d_head:(h + 4) * d_head])
        q4 = q4.astype(jnp.bfloat16).astype(jnp.float32)
        for i in range(4):
            for b in range(n_batch):
                qb_v[b * n_heads + h + i] = q4[
                    8 * b:8 * b + 8, i * d_head:(i + 1) * d_head
                ]

    cp_xa.wait()
    cp_wqa.wait()
    cp_wuk.wait()
    xa = _rows_per_batch(xa_v)
    wqa32 = wqa_v.bitcast(jnp.uint32)
    wuk32 = wuk_v.bitcast(jnp.uint32)
    wuv32 = wuv_v.bitcast(jnp.uint32)
    sub = jax.lax.broadcasted_iota(jnp.int32, (8, d_lat), 0)
    q_lat = [[None] * (n_heads // 8) for _ in range(n_batch)]
    for j in range(n_pairs):
        wq_pair = _head_pair(wqa32, j, d_model, n_pairs)
        wk_pair = _head_pair(wuk32, j, d_lat, n_pairs)
        for i in range(2):
            h = 2 * j + i
            q = _dot(xa, wq_pair[i]).astype(jnp.bfloat16)
            ql = _dot(q, wk_pair[i], _NT)
            for b in range(n_batch):
                part = ql[8 * b:8 * b + 8]
                prev = q_lat[b][h // 8]
                q_lat[b][h // 8] = (
                    part if prev is None else jnp.where(sub == h % 8, part, prev)
                )

    ctx_lat = []
    for b in range(n_batch):
        cp_ckv[b].wait()
        ql = jnp.concatenate(q_lat[b], axis=0).astype(jnp.bfloat16)
        s = _dot(ql, ckv_v[b], _NT) * scale
        m = jnp.max(s, axis=-1, keepdims=True)
        p = jnp.exp(s - m)
        l = jnp.sum(p, axis=-1, keepdims=True)
        ctx_lat.append(_dot(p.astype(jnp.bfloat16), ckv_v[b]) / l)

    cp_wuv.wait()
    row = jax.lax.broadcasted_iota(jnp.int32, (16, d_head), 0) % 8
    for j in range(n_pairs):
        g = (2 * j) // 8
        lhs = jnp.concatenate(
            [ctx_lat[b][8 * g:8 * g + 8] for b in range(n_batch)], axis=0
        ).astype(jnp.bfloat16)
        wv_pair = _head_pair(wuv32, j, d_lat, n_pairs)
        for i in range(2):
            h = 2 * j + i
            ctxa_v[h] = jnp.where(row == h % 8, _dot(lhs, wv_pair[i]), 0.0)

    def step_fn(step, carry):
        slot = step % _NBUF
        q = qb_v[step].astype(jnp.bfloat16)
        cp_k(step, slot).wait()
        s = _dot(q, k_v[slot], _NT) * scale
        m = jnp.max(s, axis=-1, keepdims=True)
        p = jnp.exp(s - m)
        l = jnp.sum(p, axis=-1, keepdims=True)
        cp_v(step, slot).wait()
        o = _dot(p.astype(jnp.bfloat16), v_v[slot]) / l
        rows = pl.ds(pl.multiple_of((step // n_heads) * 8, 8), 8)
        ctxb_v[step % n_heads, rows, :] = o

        @pl.when(step + _NBUF < n_steps)
        def _():
            cp_k(step + _NBUF, slot).start()
            cp_v(step + _NBUF, slot).start()

        @pl.when(step + _NBUF == n_steps)
        def _():
            for which in range(2):
                for c in range(_WO_CHUNKS):
                    cp_wo(which, c).start()

        return carry

    jax.lax.fori_loop(0, n_steps, step_fn, 0)

    def project(which, ctx_v, wo_v):
        acc = jnp.zeros((16, d_model), jnp.float32)
        for c in range(_WO_CHUNKS):
            heads = range(c * heads_per_chunk, (c + 1) * heads_per_chunk)
            lhs = jnp.concatenate([ctx_v[h] for h in heads], axis=1)
            cp_wo(which, c).wait()
            acc += _dot(
                lhs.astype(jnp.bfloat16),
                wo_v[c * rows_per_chunk:(c + 1) * rows_per_chunk, :],
            )
        return acc

    acc_a = project(0, ctxa_v, woa_v)
    out_a = [
        jnp.sum(acc_a[8 * b:8 * b + 8], axis=0, keepdims=True)
        for b in range(n_batch)
    ]
    acc_b = project(1, ctxb_v, wob_v)
    for b in range(n_batch):
        out_ref[b] = jnp.concatenate(
            [out_a[b], acc_b[8 * b:8 * b + 1]], axis=1
        ).astype(out_ref.dtype)


@jax.jit
def pallas_concat_heads__compressed_kv_cla__gqa_block_cached__decode_kernel(
    A_x: jax.Array,
    A_c_kv: jax.Array,
    A_w_q: jax.Array,
    A_w_uk: jax.Array,
    A_w_uv: jax.Array,
    A_w_o: jax.Array,
    B_x: jax.Array,
    B_k_cache: jax.Array,
    B_v_cache: jax.Array,
    B_wq: jax.Array,
    B_wo: jax.Array,
):
    n_batch, n_q, d_model = A_x.shape
    _, n_heads, n_kv, d_head = B_k_cache.shape
    assert n_batch == 2 and n_q == 1 and B_x.shape == A_x.shape
    assert A_w_q.shape[1:] == (n_heads, d_head) and n_heads % 8 == 0
    assert B_wq.shape == (d_model, n_heads * d_head)

    wqa = A_w_q.reshape(-1, d_head)
    wuk = A_w_uk.reshape(-1, d_head)
    wuv = A_w_uv.reshape(-1, d_head)
    woa = A_w_o.reshape(-1, d_model)

    def vmem_like(x):
        return pltpu.VMEM(x.shape, x.dtype)

    hbm = pl.BlockSpec(memory_space=pltpu.HBM)
    return pl.pallas_call(
        _kernel,
        in_specs=[hbm] * 11,
        out_specs=pl.BlockSpec(memory_space=pltpu.VMEM),
        out_shape=jax.ShapeDtypeStruct((n_batch, n_q, 2 * d_model), A_x.dtype),
        scratch_shapes=[
            vmem_like(A_x),
            vmem_like(B_x),
            vmem_like(A_c_kv),
            vmem_like(wqa),
            vmem_like(wuk),
            vmem_like(wuv),
            vmem_like(woa),
            vmem_like(B_wq),
            vmem_like(B_wo),
            pltpu.VMEM((_NBUF, n_kv, d_head), B_k_cache.dtype),
            pltpu.VMEM((_NBUF, n_kv, d_head), B_v_cache.dtype),
            pltpu.VMEM((n_batch * n_heads, 8, d_head), jnp.float32),
            pltpu.VMEM((n_heads, 16, d_head), jnp.float32),
            pltpu.VMEM((n_heads, 16, d_head), jnp.float32),
            pltpu.SemaphoreType.DMA((6 + n_batch,)),
            pltpu.SemaphoreType.DMA((2 * _WO_CHUNKS,)),
            pltpu.SemaphoreType.DMA((_NBUF,)),
            pltpu.SemaphoreType.DMA((_NBUF,)),
        ],
        compiler_params=pltpu.CompilerParams(
            vmem_limit_bytes=100 * 1024 * 1024,
        ),
    )(A_x, A_c_kv, wqa, wuk, wuv, woa, B_x, B_k_cache, B_v_cache, B_wq, B_wo)
```

```python
import jax
import jax.numpy as jnp
import jax.experimental.pallas as pl
import jax.experimental.pallas.tpu as pltpu

_ON = ("qb", "qa", "att", "uv", "B", "wo")
_P = {'nobc': True}

_STREAMS = 8
_ROUNDS = 32
_A_CHUNK = 512
_THREADS = _P.get("thr", (0, 1, 0, 1, 0, 1, 0, 1))

_NT = (((1,), (1,)), ((), ()))
_NN = (((1,), (0,)), ((), ()))


def _dot(a, b, dims=_NN):
    return jax.lax.dot_general(a, b, dims, preferred_element_type=jnp.float32)


def _rows_per_batch(x_ref):
    n = x_ref.shape[-1]
    x = x_ref[...].astype(jnp.float32)
    rows = [jnp.broadcast_to(x[b:b + 1], (8, n)) for b in range(2)]
    return jnp.concatenate(rows, axis=0).astype(jnp.bfloat16)


def _head_pair(w32_ref, j, n_pairs):
    w = w32_ref[pl.ds(j, w32_ref.shape[0] // n_pairs, stride=n_pairs), :]
    lo = pltpu.bitcast(w << 16, jnp.float32)
    hi = pltpu.bitcast(w & jnp.uint32(0xFFFF0000), jnp.float32)
    return lo.astype(jnp.bfloat16), hi.astype(jnp.bfloat16)


def _kernel(
    xa_hbm, ckv_hbm, wqa_hbm, wuk_hbm, wuv_hbm, woa_hbm,
    xb_hbm, k_hbm, v_hbm, wqb_hbm, wob_hbm,
    out_ref,
    xa_v, xb_v, ckv_v, wqa_v, wuk_v, wuv_v, wqb_v, woa_v, wob_v, k_v, v_v,
    qb_v, lat_v, s_v, p_v, ctx_v,
    w_sem, wo_sem, k_sem, v_sem,
):
    n_bh, n_kv, d_head = k_hbm.shape
    n_batch, d_model = xa_hbm.shape
    n_heads = n_bh // n_batch
    d_lat = ckv_hbm.shape[-1]
    n_pairs = n_heads // 2
    n_groups = n_bh // _STREAMS
    scale = d_head ** -0.5
    half = _STREAMS // 2

    def start(pieces):
        for (src, dst, sem), thread in zip(pieces, _THREADS, strict=True):
            pltpu.make_async_copy(src, dst, sem).start(priority=thread)

    def row_pieces(src, dst, sem, r, n_streams):
        per_stream = src.shape[0] // n_streams
        n = per_stream // _ROUNDS
        out = []
        for s in range(n_streams):
            rows = pl.ds(pl.multiple_of(s * per_stream + r * n, n), n)
            out.append((src.at[rows], dst.at[rows], sem))
        return out

    def interleave(a, b):
        return [x for pair in zip(a, b) for x in pair]

    def round_qa(r):
        start(
            row_pieces(wqa_hbm.bitcast(jnp.uint32), wqa_v, w_sem.at[0], r, half)
            + row_pieces(wuk_hbm.bitcast(jnp.uint32), wuk_v, w_sem.at[0], r, half)
        )

    def round_qb(r):
        per_stream = wqb_hbm.shape[0] // half
        cols = wqb_hbm.shape[1] // 2
        pieces = []
        for s in range(half):
            at = (
                pl.ds(pl.multiple_of(s * per_stream + (r // 2) * 8, 8), 8),
                pl.ds(pl.multiple_of((r % 2) * cols, cols), cols),
            )
            pieces.append((wqb_hbm.at[at], wqb_v.at[at], w_sem.at[1]))
        start(
            pieces
            + row_pieces(wuv_hbm.bitcast(jnp.uint32), wuv_v, w_sem.at[1], r, half)
        )

    def round_ckv(r):
        start(row_pieces(ckv_hbm, ckv_v, w_sem.at[2], r, _STREAMS))

    def round_cache(src, dst, sem, g, r):
        n = n_kv // _ROUNDS
        rows = pl.ds(pl.multiple_of(r * n, n), n)
        start([
            (src.at[g * _STREAMS + s, rows], dst.at[g % 2, s, rows], sem.at[g % 2])
            for s in range(_STREAMS)
        ])

    def round_kv(r):
        block, r = r // _ROUNDS, r % _ROUNDS
        g = block // 2
        pl.when(block % 2 == 0)(lambda: round_cache(k_hbm, k_v, k_sem, g, r))
        pl.when(block % 2 == 1)(lambda: round_cache(v_hbm, v_v, v_sem, g, r))

    rounds_per_head = _ROUNDS * half // n_heads

    def round_wo(r):
        sem = wo_sem.at[r // rounds_per_head]
        start(
            row_pieces(woa_hbm, woa_v, sem, r, half)
            + row_pieces(wob_hbm, wob_v, sem, r, half)
        )

    segments = []
    for n, fn in (
        (_ROUNDS, round_qa), (_ROUNDS, round_qb), (_ROUNDS, round_ckv),
        (2 * n_groups * _ROUNDS, round_kv), (_ROUNDS, round_wo),
    ):
        first = segments[-1][1] if segments else 0
        segments.append((first, first + n, fn))
    n_rounds = segments[-1][1]

    def issue(lo, hi, bounds):
        live = [s for s in segments if s[0] < bounds[1] and bounds[0] < s[1]]

        def one(r, carry):
            for first, end, fn in live:
                if len(live) == 1:
                    fn(r - first)
                else:
                    pl.when((r >= first) & (r < end))(
                        lambda first=first, fn=fn: fn(r - first)
                    )
            return carry

        jax.lax.fori_loop(lo, hi, one, 0)

    class Pace:
        def __init__(self, first, end, steps):
            self.first, self.end, self.steps = first, min(end, n_rounds), steps
            self.num = end - first

        def __call__(self, step):
            lo = self.first + step * self.num // self.steps
            hi = self.first + (step + 1) * self.num // self.steps
            issue(
                jnp.minimum(lo, self.end), jnp.minimum(hi, self.end),
                (self.first, self.end),
            )

    def wait_all(dst, sem):
        pltpu.make_async_copy(dst, dst, sem).wait()

    r0 = _P.get("r0", 44)
    r1 = r0 + _P.get("qa", 48)
    r2 = r1 + _P.get("qb", 16)
    r3 = r2 + _P.get("att", 48)
    r4 = r3 + _P.get("uv", 16)
    r5 = r4 + _P.get("B", 480)
    assert r5 >= n_rounds

    x_copies = [
        pltpu.make_async_copy(xa_hbm, xa_v, w_sem.at[0]),
        pltpu.make_async_copy(xb_hbm, xb_v, w_sem.at[0]),
    ]
    for cp in x_copies:
        cp.start()
    issue(0, r0, (0, r0))

    for cp in x_copies:
        cp.wait()
    wait_all(wqa_v, w_sem.at[0])
    wait_all(wuk_v, w_sem.at[0])
    xa = _rows_per_batch(xa_v)
    pace = Pace(r0, r1, n_pairs)

    @pl.loop(0, n_pairs)
    def _(j):
        if "qa" in _ON:
            wq_pair = _head_pair(wqa_v, j, n_pairs)
            wk_pair = _head_pair(wuk_v, j, n_pairs)
            for i in range(2):
                q = _dot(xa, wq_pair[i]).astype(jnp.bfloat16)
                ql = _dot(q, wk_pair[i], _NT)
                for b in range(n_batch):
                    lat_v[b, pl.ds(2 * j + i, 1), :] = ql[8 * b:8 * b + 1]
        pace(j)

    wait_all(wqb_v, w_sem.at[1])
    wait_all(wuv_v, w_sem.at[1])
    xb = _rows_per_batch(xb_v)
    pace = Pace(r1, r2, n_heads // 4)

    @pl.loop(0, n_heads // 4)
    def _(g):
        if "qb" in _ON:
            cols = pl.ds(pl.multiple_of(g * 4 * d_head, 4 * d_head), 4 * d_head)
            q4 = _dot(xb, wqb_v[:, cols])
            q4 = q4.astype(jnp.bfloat16).astype(jnp.float32)
            for i in range(4):
                for b in range(n_batch):
                    qb_v[b * n_heads + g * 4 + i] = q4[
                        8 * b:8 * b + 8, i * d_head:(i + 1) * d_head
                    ]
        pace(g)

    n_chunks = n_kv // _A_CHUNK
    wait_all(ckv_v, w_sem.at[2])
    pace = Pace(r2, r3, n_batch * n_chunks * 3)

    @pl.loop(0, n_batch)
    def _(b):
        ql = lat_v[b].astype(jnp.bfloat16)

        def keys(c):
            first = pl.multiple_of(b * n_kv + c * _A_CHUNK, _A_CHUNK)
            return ckv_v[pl.ds(first, _A_CHUNK), :]

        def scores(c, m):
            if "att" in _ON:
                s = _dot(ql, keys(c), _NT) * scale
                s_v[c] = s
                m = jnp.maximum(m, jnp.max(s, axis=-1, keepdims=True))
            step = (b * n_chunks * 3) + 2 * c
            pace(step)
            pace(step + 1)
            return m

        m = jax.lax.fori_loop(
            0, n_chunks, scores, jnp.full((n_heads, 1), -jnp.inf, jnp.float32)
        )

        def values(c, carry):
            l, acc = carry
            if "att" in _ON:
                p = jnp.exp(s_v[c] - m)
                l = l + jnp.sum(p, axis=-1, keepdims=True)
                acc = acc + _dot(p.astype(jnp.bfloat16), keys(c))
            pace((b * 3 + 2) * n_chunks + c)
            return l, acc

        l, acc = jax.lax.fori_loop(
            0, n_chunks, values,
            (jnp.zeros((n_heads, 1), jnp.float32),
             jnp.zeros((n_heads, d_lat), jnp.float32)),
        )
        lat_v[b] = acc / l

    pace = Pace(r3, r4, n_pairs)

    @pl.loop(0, n_pairs)
    def _(j):
        if "uv" in _ON:
            wv_pair = _head_pair(wuv_v, j, n_pairs)
            for i in range(2):
                h = 2 * j + i
                lhs = jnp.concatenate(
                    [jnp.broadcast_to(lat_v[b, pl.ds(h, 1), :], (8, d_lat))
                     for b in range(n_batch)], axis=0,
                ).astype(jnp.bfloat16)
                ctx_v[0, h] = _dot(lhs, wv_pair[i])
        pace(j)

    pace = Pace(r4, r5, 2 * n_bh)

    @pl.loop(0, n_groups)
    def _(g):
        slot = g % 2
        wait_all(k_v.at[slot], k_sem.at[slot])

        @pl.loop(0, _STREAMS)
        def _(i):
            if "B" in _ON:
                q = qb_v[g * _STREAMS + i].astype(jnp.bfloat16)
                s = _dot(q, k_v[slot, i], _NT) * scale
                p = jnp.exp(s - jnp.max(s, axis=-1, keepdims=True))
                p_v[i] = p / jnp.sum(p, axis=-1, keepdims=True)
            pace(2 * g * _STREAMS + i)

        wait_all(v_v.at[slot], v_sem.at[slot])

        @pl.loop(0, _STREAMS)
        def _(i):
            if "B" in _ON:
                bh = g * _STREAMS + i
                o = _dot(p_v[i].astype(jnp.bfloat16), v_v[slot, i])
                rows = pl.ds(pl.multiple_of((bh // n_heads) * 8, 8), 8)
                ctx_v[1, bh % n_heads, rows, :] = o
            pace((2 * g + 1) * _STREAMS + i)

    heads_per_stream = n_heads // half

    def project(i, accs):
        wait_all(woa_v.at[pl.ds(0, 2 * half * d_head)], wo_sem.at[i])
        if "wo" not in _ON:
            return accs
        out = []
        for which, wo_v in enumerate((woa_v, wob_v)):
            acc = accs[which]
            for s in range(half):
                h = s * heads_per_stream + i
                rows = pl.ds(pl.multiple_of(h * d_head, d_head), d_head)
                acc = acc + _dot(ctx_v[which, h].astype(jnp.bfloat16), wo_v[rows, :])
            out.append(acc)
        return tuple(out)

    zero = jnp.zeros((16, d_model), jnp.float32)
    accs = jax.lax.fori_loop(0, heads_per_stream, project, (zero, zero))
    out = jnp.concatenate(accs, axis=1)
    out = jnp.concatenate([out[8 * b:8 * b + 1] for b in range(n_batch)], axis=0)
    out_ref[...] = out.astype(out_ref.dtype)


@jax.jit
def pallas_concat_heads__compressed_kv_cla__gqa_block_cached__decode_kernel(
    A_x, A_c_kv, A_w_q, A_w_uk, A_w_uv, A_w_o, B_x, B_k_cache, B_v_cache, B_wq, B_wo,
):
    n_batch, n_q, d_model = A_x.shape
    _, n_heads, n_kv, d_head = B_k_cache.shape
    d_lat = A_c_kv.shape[-1]

    xa = A_x.reshape(n_batch, d_model)
    xb = B_x.reshape(n_batch, d_model)
    ckv = A_c_kv.reshape(-1, d_lat)
    wqa = A_w_q.reshape(-1, d_head)
    wuk = A_w_uk.reshape(-1, d_head)
    wuv = A_w_uv.reshape(-1, d_head)
    woa = A_w_o.reshape(-1, d_model)
    k = B_k_cache.reshape(-1, n_kv, d_head)
    v = B_v_cache.reshape(-1, n_kv, d_head)

    def vmem_like(x):
        return pltpu.VMEM(x.shape, x.dtype)

    def vmem_words(x):
        return pltpu.VMEM((x.shape[0] // 2, x.shape[1]), jnp.uint32)

    hbm = pl.BlockSpec(memory_space=pltpu.HBM)
    out = pl.pallas_call(
        _kernel,
        in_specs=[hbm] * 11,
        out_specs=pl.BlockSpec(memory_space=pltpu.VMEM),
        out_shape=jax.ShapeDtypeStruct((n_batch, 2 * d_model), A_x.dtype),
        scratch_shapes=[
            vmem_like(xa),
            vmem_like(xb),
            vmem_like(ckv),
            vmem_words(wqa),
            vmem_words(wuk),
            vmem_words(wuv),
            vmem_like(B_wq),
            vmem_like(woa),
            vmem_like(B_wo),
            pltpu.VMEM((2, _STREAMS, n_kv, d_head), k.dtype),
            pltpu.VMEM((2, _STREAMS, n_kv, d_head), v.dtype),
            pltpu.VMEM((n_batch * n_heads, 8, d_head), jnp.float32),
            pltpu.VMEM((n_batch, n_heads, d_lat), jnp.float32),
            pltpu.VMEM((n_kv // _A_CHUNK, n_heads, _A_CHUNK), jnp.float32),
            pltpu.VMEM((_STREAMS, 8, n_kv), jnp.float32),
            pltpu.VMEM((2, n_heads, 16, d_head), jnp.float32),
            pltpu.SemaphoreType.DMA((3,)),
            pltpu.SemaphoreType.DMA((2 * n_heads // _STREAMS,)),
            pltpu.SemaphoreType.DMA((2,)),
            pltpu.SemaphoreType.DMA((2,)),
        ],
        compiler_params=pltpu.CompilerParams(
            vmem_limit_bytes=100 * 1024 * 1024,
            disable_bounds_checks=_P.get("nobc", False),
        ),
    )(xa, ckv, wqa, wuk, wuv, woa, xb, k, v, B_wq, B_wo)
    return out.reshape(n_batch, n_q, 2 * d_model)
```

```python
import jax
import jax.numpy as jnp
import jax.experimental.pallas as pl
import jax.experimental.pallas.tpu as pltpu

_ON = ("qb", "qa", "att", "uv", "B", "wo")
_P = {}

_STREAMS = 8
_ROUNDS = 32
_BLOCK_SEMS = 4
_A_CHUNK = 512
_TAIL = _P.get("tail", (2, 1, 1))

_NT = (((1,), (1,)), ((), ()))
_NN = (((1,), (0,)), ((), ()))


def _dot(a, b, dims=_NN):
    return jax.lax.dot_general(a, b, dims, preferred_element_type=jnp.float32)


def _rows_per_batch(x_ref):
    n = x_ref.shape[-1]
    x = x_ref[...].astype(jnp.float32)
    rows = [jnp.broadcast_to(x[b:b + 1], (8, n)) for b in range(2)]
    return jnp.concatenate(rows, axis=0).astype(jnp.bfloat16)


def _head_pair(w32_ref, j, n_pairs):
    w = w32_ref[pl.ds(j, w32_ref.shape[0] // n_pairs, stride=n_pairs), :]
    lo = pltpu.bitcast(w << 16, jnp.float32)
    hi = pltpu.bitcast(w & jnp.uint32(0xFFFF0000), jnp.float32)
    return lo.astype(jnp.bfloat16), hi.astype(jnp.bfloat16)


def _aligned(first, size):
    return pl.ds(pl.multiple_of(first, size), size)


def _interleave(a, b):
    return [x for pair in zip(a, b, strict=True) for x in pair]


def _wait_filled(dst, sem):
    pltpu.make_async_copy(dst, dst, sem).wait()


def _kernel(
    xa_hbm, ckv_hbm, wqa_hbm, wuk_hbm, wuv_hbm, woa_hbm,
    xb_hbm, k_hbm, v_hbm, wqb_hbm, wob_hbm,
    out_ref,
    xa_v, xb_v, ckv_v, wqa_v, wuk_v, wuv_v, wqb_v, woa_v, wob_v, k_v, v_v,
    qb_v, lat_v, s_v, p_v, ctx_v,
    sems,
):
    _, n_groups, n_kv, d_head = k_hbm.shape
    n_batch, d_model = xa_hbm.shape
    n_bh = _STREAMS * n_groups
    n_heads = n_bh // n_batch
    n_pairs = n_heads // 2
    d_lat = ckv_hbm.shape[-1]
    n_chunks = n_kv // _A_CHUNK
    scale = d_head ** -0.5
    half = _STREAMS // 2
    heads_per_stream = n_heads // half

    first_kv = 3
    wo_block = first_kv + 2 * n_groups

    def block_sem(n):
        return sems.at[n % _BLOCK_SEMS]

    def start(pieces, threads=(0, 1) * half):
        for (src, dst, sem), thread in zip(pieces, threads, strict=True):
            pltpu.make_async_copy(src, dst, sem).start(priority=thread)

    def row_pieces(src, dst, sem, r, n_streams):
        n = src.shape[0] // (n_streams * _ROUNDS)
        rows = [_aligned((s * _ROUNDS + r) * n, n) for s in range(n_streams)]
        return [(src.at[x], dst.at[x], sem) for x in rows]

    def words(ref):
        return ref.bitcast(jnp.uint32)

    def round_qa(r, **kwargs):
        start(_interleave(
            row_pieces(words(wqa_hbm), wqa_v, block_sem(0), r, half),
            row_pieces(words(wuk_hbm), wuk_v, block_sem(0), r, half),
        ), **kwargs)

    def round_qb(r):
        per_stream = wqb_hbm.shape[0] // half
        cols = _aligned((r % 2) * (wqb_hbm.shape[1] // 2), wqb_hbm.shape[1] // 2)
        rows = [_aligned(s * per_stream + (r // 2) * 8, 8) for s in range(half)]
        start(_interleave(
            [(wqb_hbm.at[x, cols], wqb_v.at[x, cols], block_sem(1)) for x in rows],
            row_pieces(words(wuv_hbm), wuv_v, block_sem(1), r, half),
        ))

    def round_ckv(r):
        start(row_pieces(ckv_hbm, ckv_v, block_sem(2), r, _STREAMS))

    def round_kv(r):
        block, r = r // _ROUNDS, r % _ROUNDS
        g = block // 2
        sem = block_sem(first_kv + block)
        rows = _aligned(r * (n_kv // _ROUNDS), n_kv // _ROUNDS)

        def cache(src, dst):
            start([
                (src.at[s, g, rows], dst.at[g % 2, s, rows], sem)
                for s in range(_STREAMS)
            ])

        pl.when(block % 2 == 0)(lambda: cache(k_hbm, k_v))
        pl.when(block % 2 == 1)(lambda: cache(v_hbm, v_v))

    per_head = _ROUNDS // heads_per_stream
    last = _ROUNDS - per_head
    tail_first = [sum(_TAIL[:i]) for i in range(len(_TAIL))]
    assert sum(_TAIL) == half and heads_per_stream == 8

    def wo_sem(i):
        if isinstance(i, int):
            return sems.at[i if i >= _BLOCK_SEMS else (wo_block + i) % _BLOCK_SEMS]
        return sems.at[jnp.where(i >= _BLOCK_SEMS, i, (wo_block + i) % _BLOCK_SEMS)]

    def round_wo(r):
        head = r // per_head
        n = d_head // per_head
        in_tail = r >= last
        tail_sem = _BLOCK_SEMS - 1 + sum(
            (r - last >= s).astype(jnp.int32) for s in tail_first
        )
        sem_a = wo_sem(jnp.where(head < 6, 0, 2))
        sem_b = wo_sem(jnp.where(
            head < 4, 0, jnp.where(head < 6, 1, jnp.where(in_tail, tail_sem, 3))
        ))
        pieces = []
        for s in range(half):
            at = (s, head, _aligned((r % per_head) * n, n))
            pieces.append((woa_hbm.at[at], woa_v.at[at], sem_a))
            at = (
                jnp.where(in_tail, r - last, s),
                head,
                _aligned(jnp.where(in_tail, s, r % per_head) * n, n),
            )
            pieces.append((wob_hbm.at[at], wob_v.at[at], sem_b))
        start(pieces)

    segments = []
    for n, fn in (
        (1, round_qa), (1, round_qb), (1, round_ckv),
        (2 * n_groups, round_kv), (1, round_wo),
    ):
        first = segments[-1][1] if segments else 0
        segments.append((first, first + n * _ROUNDS, fn))
    n_rounds = segments[-1][1]

    def issue(lo, hi, bounds):
        live = [s for s in segments if s[0] < bounds[1] and bounds[0] < s[1]]

        def one(r, carry):
            for first, end, fn in live:
                if len(live) == 1:
                    fn(r - first)
                else:
                    pl.when((r >= first) & (r < end))(
                        lambda first=first, fn=fn: fn(r - first)
                    )
            return carry

        jax.lax.fori_loop(lo, hi, one, 0)

    def pacer(first, n, steps):
        end = min(first + n, n_rounds)

        def pace(step):
            lo = first + step * n // steps
            hi = first + (step + 1) * n // steps
            issue(jnp.minimum(lo, end), jnp.minimum(hi, end), (first, end))

        return pace

    n_qa, n_qb, n_att, n_uv, n_b = (
        _P.get("qa", 48), _P.get("qb", 16), _P.get("att", 48), _P.get("uv", 16),
        _P.get("B", 480),
    )
    at_qa = _P.get("r0", 44)
    at_qb = at_qa + n_qa
    at_att = at_qb + n_qb
    at_uv = at_att + n_att
    at_b = at_uv + n_uv
    waited = [at_qa, at_qb, at_att] + [
        at_b + i * _STREAMS * n_b // (2 * n_bh) for i in range(2 * n_groups + 1)
    ]
    for n in range(wo_block):
        assert (n + 1) * _ROUNDS <= waited[n]
        assert waited[n + (n >= first_kv)] <= (n + _BLOCK_SEMS) * _ROUNDS
    for i, head in enumerate((0, 4, 6, 6)):
        assert waited[wo_block + i - _BLOCK_SEMS] <= wo_block * _ROUNDS + head * per_head
    assert waited[-1] >= n_rounds

    n_fill = _P.get("fill", 3)

    @pl.loop(0, n_fill)
    def _(r):
        round_qa(r, threads=(1,) * _STREAMS)

    x_copies = [
        pltpu.make_async_copy(xa_hbm, xa_v, block_sem(0)),
        pltpu.make_async_copy(xb_hbm, xb_v, block_sem(0)),
    ]
    for cp in x_copies:
        cp.start()
    issue(n_fill, at_qa, (n_fill, at_qa))

    for cp in x_copies:
        cp.wait()
    _wait_filled(wqa_v, block_sem(0))
    _wait_filled(wuk_v, block_sem(0))
    xa = _rows_per_batch(xa_v)
    pace = pacer(at_qa, n_qa, n_pairs)

    @pl.loop(0, n_pairs)
    def _(j):
        if "qa" in _ON:
            wq_pair = _head_pair(wqa_v, j, n_pairs)
            wk_pair = _head_pair(wuk_v, j, n_pairs)
            for i in range(2):
                q = _dot(xa, wq_pair[i]).astype(jnp.bfloat16)
                ql = _dot(q, wk_pair[i], _NT)
                for b in range(n_batch):
                    lat_v[b, pl.ds(2 * j + i, 1), :] = ql[8 * b:8 * b + 1]
        pace(j)

    _wait_filled(wqb_v, block_sem(1))
    _wait_filled(wuv_v, block_sem(1))
    xb = _rows_per_batch(xb_v)
    pace = pacer(at_qb, n_qb, n_heads // 4)

    @pl.loop(0, n_heads // 4)
    def _(j):
        if "qb" in _ON:
            q4 = _dot(xb, wqb_v[:, _aligned(j * 4 * d_head, 4 * d_head)])
            q4 = q4.astype(jnp.bfloat16).astype(jnp.float32)
            for i in range(4):
                for b in range(n_batch):
                    qb_v[b * n_heads + j * 4 + i] = q4[
                        8 * b:8 * b + 8, i * d_head:(i + 1) * d_head
                    ]
        pace(j)

    _wait_filled(ckv_v, block_sem(2))
    pace = pacer(at_att, n_att, n_batch * n_chunks * 3)

    @pl.loop(0, n_batch)
    def _(b):
        ql = lat_v[b].astype(jnp.bfloat16)

        def keys(c):
            return ckv_v[_aligned(b * n_kv + c * _A_CHUNK, _A_CHUNK), :]

        def scores(c, m):
            if "att" in _ON:
                s = _dot(ql, keys(c), _NT) * scale
                s_v[c] = s
                m = jnp.maximum(m, jnp.max(s, axis=-1, keepdims=True))

            @pl.loop(0, 2)
            def _(i):
                pace(b * 3 * n_chunks + 2 * c + i)

            return m

        m = jax.lax.fori_loop(
            0, n_chunks, scores, jnp.full((n_heads, 1), -jnp.inf, jnp.float32)
        )

        def values(c, carry):
            l, acc = carry
            if "att" in _ON:
                p = jnp.exp(s_v[c] - m)
                l = l + jnp.sum(p, axis=-1, keepdims=True)
                acc = acc + _dot(p.astype(jnp.bfloat16), keys(c))
            pace((b * 3 + 2) * n_chunks + c)
            return l, acc

        l, acc = jax.lax.fori_loop(
            0, n_chunks, values,
            (jnp.zeros((n_heads, 1), jnp.float32),
             jnp.zeros((n_heads, d_lat), jnp.float32)),
        )
        lat_v[b] = acc / l

    pace = pacer(at_uv, n_uv, n_pairs)

    @pl.loop(0, n_pairs)
    def _(j):
        if "uv" in _ON:
            wv_pair = _head_pair(wuv_v, j, n_pairs)
            for i in range(2):
                h = 2 * j + i
                lhs = jnp.concatenate(
                    [jnp.broadcast_to(lat_v[b, pl.ds(h, 1), :], (8, d_lat))
                     for b in range(n_batch)], axis=0,
                ).astype(jnp.bfloat16)
                ctx_v[0, h] = _dot(lhs, wv_pair[i])
        pace(j)

    pace = pacer(at_b, n_b, 2 * n_bh)

    @pl.loop(0, n_groups)
    def _(g):
        slot = g % 2
        _wait_filled(k_v.at[slot], block_sem(first_kv + 2 * g))

        @pl.loop(0, _STREAMS)
        def _(i):
            if "B" in _ON:
                q = qb_v[i * n_groups + g].astype(jnp.bfloat16)
                s = _dot(q, k_v[slot, i], _NT) * scale
                p = jnp.exp(s - jnp.max(s, axis=-1, keepdims=True))
                p_v[i] = p / jnp.sum(p, axis=-1, keepdims=True)
            pace(2 * g * _STREAMS + i)

        _wait_filled(v_v.at[slot], block_sem(first_kv + 2 * g + 1))

        @pl.loop(0, _STREAMS)
        def _(i):
            if "B" in _ON:
                bh = i * n_groups + g
                o = _dot(p_v[i].astype(jnp.bfloat16), v_v[slot, i])
                ctx_v[1, bh % n_heads, _aligned((bh // n_heads) * 8, 8), :] = o
            pace((2 * g + 1) * _STREAMS + i)

    def project(acc, which, heads, streams=range(half)):
        wo_v = (woa_v, wob_v)[which]
        if "wo" not in _ON:
            return acc
        for i in heads:
            for s in streams:
                ctx = ctx_v[which, s * heads_per_stream + i].astype(jnp.bfloat16)
                acc = acc + _dot(ctx, wo_v[s, i])
        return acc

    def project_first(which, n):
        return jax.lax.fori_loop(
            0, n // 2,
            lambda i, acc: project(acc, which, (2 * i, 2 * i + 1)),
            jnp.zeros((16, d_model), jnp.float32),
        )

    _wait_filled(woa_v.at[:, 0:6], wo_sem(0))
    _wait_filled(wob_v.at[:, 0:4], wo_sem(0))
    acc_a = project_first(0, 6)
    acc_b = project_first(1, 4)
    _wait_filled(wob_v.at[:, 4:6], wo_sem(1))
    acc_b = project(acc_b, 1, (4, 5))
    _wait_filled(woa_v.at[:, 6:8], wo_sem(2))
    acc_a = project(acc_a, 0, (6, 7))
    _wait_filled(wob_v.at[:, 6], wo_sem(3))
    acc_b = project(acc_b, 1, (6,))
    for i, (s, n) in enumerate(zip(tail_first, _TAIL)):
        _wait_filled(wob_v.at[s:s + n, 7], wo_sem(_BLOCK_SEMS + i))
        acc_b = project(acc_b, 1, (7,), range(s, s + n))

    out = jnp.concatenate([acc_a, acc_b], axis=1)
    out = jnp.concatenate([out[8 * b:8 * b + 1] for b in range(n_batch)], axis=0)
    out_ref[...] = out.astype(out_ref.dtype)


@jax.jit
def pallas_concat_heads__compressed_kv_cla__gqa_block_cached__decode_kernel(
    A_x: jax.Array,
    A_c_kv: jax.Array,
    A_w_q: jax.Array,
    A_w_uk: jax.Array,
    A_w_uv: jax.Array,
    A_w_o: jax.Array,
    B_x: jax.Array,
    B_k_cache: jax.Array,
    B_v_cache: jax.Array,
    B_wq: jax.Array,
    B_wo: jax.Array,
):
    n_batch, n_q, d_model = A_x.shape
    _, n_heads, n_kv, d_head = B_k_cache.shape
    d_lat = A_c_kv.shape[-1]
    assert n_batch == 2 and n_q == 1 and B_x.shape == A_x.shape
    assert A_c_kv.shape[1] == n_kv and A_w_q.shape[1:] == (n_heads, d_head)
    assert B_wq.shape == (d_model, n_heads * d_head)

    wo_shape = (_STREAMS // 2, 2 * n_heads // _STREAMS, d_head, d_model)
    xa = A_x.reshape(n_batch, d_model)
    xb = B_x.reshape(n_batch, d_model)
    ckv = A_c_kv.reshape(-1, d_lat)
    wqa = A_w_q.reshape(-1, d_head)
    wuk = A_w_uk.reshape(-1, d_head)
    wuv = A_w_uv.reshape(-1, d_head)
    woa = A_w_o.reshape(wo_shape)
    wob = B_wo.reshape(wo_shape)
    k = B_k_cache.reshape(_STREAMS, -1, n_kv, d_head)
    v = B_v_cache.reshape(_STREAMS, -1, n_kv, d_head)

    def vmem_like(x):
        return pltpu.VMEM(x.shape, x.dtype)

    def vmem_words(x):
        return pltpu.VMEM((x.shape[0] // 2, x.shape[1]), jnp.uint32)

    out = pl.pallas_call(
        _kernel,
        in_specs=[pl.BlockSpec(memory_space=pltpu.HBM)] * 11,
        out_specs=pl.BlockSpec(memory_space=pltpu.VMEM),
        out_shape=jax.ShapeDtypeStruct((n_batch, 2 * d_model), A_x.dtype),
        scratch_shapes=[
            vmem_like(xa),
            vmem_like(xb),
            vmem_like(ckv),
            vmem_words(wqa),
            vmem_words(wuk),
            vmem_words(wuv),
            vmem_like(B_wq),
            vmem_like(woa),
            vmem_like(wob),
            pltpu.VMEM((2, _STREAMS, n_kv, d_head), k.dtype),
            pltpu.VMEM((2, _STREAMS, n_kv, d_head), v.dtype),
            pltpu.VMEM((n_batch * n_heads, 8, d_head), jnp.float32),
            pltpu.VMEM((n_batch, n_heads, d_lat), jnp.float32),
            pltpu.VMEM((n_kv // _A_CHUNK, n_heads, _A_CHUNK), jnp.float32),
            pltpu.VMEM((_STREAMS, 8, n_kv), jnp.float32),
            pltpu.VMEM((2, n_heads, 16, d_head), jnp.float32),
            pltpu.SemaphoreType.DMA((_BLOCK_SEMS + len(_TAIL),)),
        ],
        compiler_params=pltpu.CompilerParams(
            vmem_limit_bytes=100 * 1024 * 1024,
            disable_bounds_checks=True,
        ),
    )(xa, ckv, wqa, wuk, wuv, woa, xb, k, v, B_wq, wob)
    return out.reshape(n_batch, n_q, 2 * d_model)
```

```python
import jax
import jax.numpy as jnp
import jax.experimental.pallas as pl
import jax.experimental.pallas.tpu as pltpu

_STREAMS = 8
_ROUNDS = 32
_BLOCK_SEMS = 4
_TAIL = (2, 1, 1)
_A_CHUNK = 512

_FILL_ROUNDS = 3
_LEAD_ROUNDS = 44
_QA_ROUNDS, _QB_ROUNDS, _ATT_ROUNDS, _UV_ROUNDS, _B_ROUNDS = 52, 12, 42, 22, 480

_NT = (((1,), (1,)), ((), ()))
_NN = (((1,), (0,)), ((), ()))


def _dot(a, b, dims=_NN):
    return jax.lax.dot_general(a, b, dims, preferred_element_type=jnp.float32)


def _rows_per_batch(x_ref):
    n = x_ref.shape[-1]
    x = x_ref[...].astype(jnp.float32)
    rows = [jnp.broadcast_to(x[b:b + 1], (8, n)) for b in range(2)]
    return jnp.concatenate(rows, axis=0).astype(jnp.bfloat16)


def _head_pair(w32_ref, j, n_pairs):
    w = w32_ref[pl.ds(j, w32_ref.shape[0] // n_pairs, stride=n_pairs), :]
    lo = pltpu.bitcast(w << 16, jnp.float32)
    hi = pltpu.bitcast(w & jnp.uint32(0xFFFF0000), jnp.float32)
    return lo.astype(jnp.bfloat16), hi.astype(jnp.bfloat16)


def _aligned(first, size):
    return pl.ds(pl.multiple_of(first, size), size)


def _interleave(a, b):
    return [x for pair in zip(a, b, strict=True) for x in pair]


def _wait_filled(dst, sem):
    pltpu.make_async_copy(dst, dst, sem).wait()


def _kernel(
    xa_hbm, ckv_hbm, wqa_hbm, wuk_hbm, wuv_hbm, woa_hbm,
    xb_hbm, k_hbm, v_hbm, wqb_hbm, wob_hbm,
    out_ref,
    xa_v, xb_v, ckv_v, wqa_v, wuk_v, wuv_v, wqb_v, woa_v, wob_v, k_v, v_v,
    qb_v, lat_v, s_v, p_v, ctx_v,
    sems,
):
    _, n_groups, n_kv, d_head = k_hbm.shape
    n_batch, d_model = xa_hbm.shape
    n_bh = _STREAMS * n_groups
    n_heads = n_bh // n_batch
    n_pairs = n_heads // 2
    d_lat = ckv_hbm.shape[-1]
    n_chunks = n_kv // _A_CHUNK
    scale = d_head ** -0.5
    half = _STREAMS // 2
    heads_per_stream = n_heads // half

    first_kv = 3
    wo_block = first_kv + 2 * n_groups

    def block_sem(n):
        return sems.at[n % _BLOCK_SEMS]

    def start(pieces, threads=(0, 1) * half):
        for (src, dst, sem), thread in zip(pieces, threads, strict=True):
            pltpu.make_async_copy(src, dst, sem).start(priority=thread)

    def row_pieces(src, dst, sem, r, n_streams):
        n = src.shape[0] // (n_streams * _ROUNDS)
        rows = [_aligned((s * _ROUNDS + r) * n, n) for s in range(n_streams)]
        return [(src.at[x], dst.at[x], sem) for x in rows]

    def words(ref):
        return ref.bitcast(jnp.uint32)

    def round_qa(r, **kwargs):
        start(_interleave(
            row_pieces(words(wqa_hbm), wqa_v, block_sem(0), r, half),
            row_pieces(words(wuk_hbm), wuk_v, block_sem(0), r, half),
        ), **kwargs)

    def round_qb(r):
        per_stream = wqb_hbm.shape[0] // half
        cols = _aligned((r % 2) * (wqb_hbm.shape[1] // 2), wqb_hbm.shape[1] // 2)
        rows = [_aligned(s * per_stream + (r // 2) * 8, 8) for s in range(half)]
        start(_interleave(
            [(wqb_hbm.at[x, cols], wqb_v.at[x, cols], block_sem(1)) for x in rows],
            row_pieces(words(wuv_hbm), wuv_v, block_sem(1), r, half),
        ))

    def round_ckv(r):
        start(row_pieces(ckv_hbm, ckv_v, block_sem(2), r, _STREAMS))

    def round_kv(r):
        block, r = r // _ROUNDS, r % _ROUNDS
        g = block // 2
        sem = block_sem(first_kv + block)
        rows = _aligned(r * (n_kv // _ROUNDS), n_kv // _ROUNDS)

        def cache(src, dst):
            start([
                (src.at[s, g, rows], dst.at[g % 2, s, rows], sem)
                for s in range(_STREAMS)
            ])

        pl.when(block % 2 == 0)(lambda: cache(k_hbm, k_v))
        pl.when(block % 2 == 1)(lambda: cache(v_hbm, v_v))

    per_head = _ROUNDS // heads_per_stream
    last = _ROUNDS - per_head
    tail_first = [sum(_TAIL[:i]) for i in range(len(_TAIL))]
    assert sum(_TAIL) == half == per_head and heads_per_stream == 8

    def wo_sem(i):
        if isinstance(i, int):
            return sems.at[i] if i >= _BLOCK_SEMS else block_sem(wo_block + i)
        return sems.at[jnp.where(i >= _BLOCK_SEMS, i, (wo_block + i) % _BLOCK_SEMS)]

    def round_wo(r):
        head = r // per_head
        n = d_head // per_head
        in_tail = r >= last
        tail_sem = _BLOCK_SEMS - 1 + sum(
            (r - last >= s).astype(jnp.int32) for s in tail_first
        )
        sem_a = wo_sem(jnp.where(head < 6, 0, 2))
        sem_b = wo_sem(jnp.where(
            head < 4, 0, jnp.where(head < 6, 1, jnp.where(in_tail, tail_sem, 3))
        ))
        pieces = []
        for s in range(half):
            at = (s, head, _aligned((r % per_head) * n, n))
            pieces.append((woa_hbm.at[at], woa_v.at[at], sem_a))
            at = (
                jnp.where(in_tail, r - last, s),
                head,
                _aligned(jnp.where(in_tail, s, r % per_head) * n, n),
            )
            pieces.append((wob_hbm.at[at], wob_v.at[at], sem_b))
        start(pieces)

    segments = []
    for n, fn in (
        (1, round_qa), (1, round_qb), (1, round_ckv),
        (2 * n_groups, round_kv), (1, round_wo),
    ):
        first = segments[-1][1] if segments else 0
        segments.append((first, first + n * _ROUNDS, fn))
    n_rounds = segments[-1][1]

    def issue(lo, hi, bounds):
        live = [s for s in segments if s[0] < bounds[1] and bounds[0] < s[1]]

        def one(r, carry):
            for first, end, fn in live:
                if len(live) == 1:
                    fn(r - first)
                else:
                    pl.when((r >= first) & (r < end))(
                        lambda first=first, fn=fn: fn(r - first)
                    )
            return carry

        jax.lax.fori_loop(lo, hi, one, 0)

    def pacer(first, n, steps):
        end = min(first + n, n_rounds)

        def pace(step):
            lo = first + step * n // steps
            hi = first + (step + 1) * n // steps
            issue(jnp.minimum(lo, end), jnp.minimum(hi, end), (first, end))

        return pace

    at_qa = _LEAD_ROUNDS
    at_qb = at_qa + _QA_ROUNDS
    at_att = at_qb + _QB_ROUNDS
    at_uv = at_att + _ATT_ROUNDS
    at_b = at_uv + _UV_ROUNDS
    waited = [at_qa, at_qb, at_att] + [
        at_b + i * _STREAMS * _B_ROUNDS // (2 * n_bh)
        for i in range(2 * n_groups + 1)
    ]
    for n in range(wo_block):
        assert (n + 1) * _ROUNDS <= waited[n]
        assert waited[n + (n >= first_kv)] <= (n + _BLOCK_SEMS) * _ROUNDS
    for i, head in enumerate((0, 4, 6, 6)):
        taken_over = wo_block * _ROUNDS + head * per_head
        assert waited[wo_block + i - _BLOCK_SEMS] <= taken_over
    assert waited[-1] >= n_rounds

    @pl.loop(0, _FILL_ROUNDS)
    def _(r):
        round_qa(r, threads=(1,) * _STREAMS)

    x_copies = [
        pltpu.make_async_copy(xa_hbm, xa_v, block_sem(0)),
        pltpu.make_async_copy(xb_hbm, xb_v, block_sem(0)),
    ]
    for cp in x_copies:
        cp.start()
    issue(_FILL_ROUNDS, at_qa, (_FILL_ROUNDS, at_qa))

    for cp in x_copies:
        cp.wait()
    _wait_filled(wqa_v, block_sem(0))
    _wait_filled(wuk_v, block_sem(0))
    xa = _rows_per_batch(xa_v)
    pace_qa = pacer(at_qa, _QA_ROUNDS, n_pairs)

    @pl.loop(0, n_pairs)
    def _(j):
        wq_pair = _head_pair(wqa_v, j, n_pairs)
        wk_pair = _head_pair(wuk_v, j, n_pairs)
        for i in range(2):
            q = _dot(xa, wq_pair[i]).astype(jnp.bfloat16)
            q_lat = _dot(q, wk_pair[i], _NT)
            for b in range(n_batch):
                lat_v[b, pl.ds(2 * j + i, 1), :] = q_lat[8 * b:8 * b + 1]
        pace_qa(j)

    _wait_filled(wqb_v, block_sem(1))
    _wait_filled(wuv_v, block_sem(1))
    xb = _rows_per_batch(xb_v)
    pace_qb = pacer(at_qb, _QB_ROUNDS, n_heads // 4)

    @pl.loop(0, n_heads // 4)
    def _(j):
        q = _dot(xb, wqb_v[:, _aligned(j * 4 * d_head, 4 * d_head)])
        for i in range(4):
            for b in range(n_batch):
                qb_v[b * n_heads + j * 4 + i] = q[
                    8 * b:8 * b + 8, i * d_head:(i + 1) * d_head
                ]
        pace_qb(j)

    _wait_filled(ckv_v, block_sem(2))
    pace_att = pacer(at_att, _ATT_ROUNDS, n_batch * n_chunks * 3)

    @pl.loop(0, n_batch)
    def _(b):
        q_lat = lat_v[b].astype(jnp.bfloat16)

        def keys(c):
            return ckv_v[_aligned(b * n_kv + c * _A_CHUNK, _A_CHUNK), :]

        def scores(c, m):
            s = _dot(q_lat, keys(c), _NT) * scale
            s_v[c] = s

            @pl.loop(0, 2)
            def _(i):
                pace_att(b * 3 * n_chunks + 2 * c + i)

            return jnp.maximum(m, jnp.max(s, axis=-1, keepdims=True))

        m = jax.lax.fori_loop(
            0, n_chunks, scores, jnp.full((n_heads, 1), -jnp.inf, jnp.float32)
        )

        def values(c, carry):
            l, acc = carry
            p = jnp.exp(s_v[c] - m)
            l = l + jnp.sum(p, axis=-1, keepdims=True)
            acc = acc + _dot(p.astype(jnp.bfloat16), keys(c))
            pace_att((b * 3 + 2) * n_chunks + c)
            return l, acc

        l, acc = jax.lax.fori_loop(
            0, n_chunks, values,
            (jnp.zeros((n_heads, 1), jnp.float32),
             jnp.zeros((n_heads, d_lat), jnp.float32)),
        )
        lat_v[b] = acc / l

    pace_uv = pacer(at_uv, _UV_ROUNDS, n_pairs)

    @pl.loop(0, n_pairs)
    def _(j):
        wv_pair = _head_pair(wuv_v, j, n_pairs)
        for i in range(2):
            h = 2 * j + i
            ctx_lat = jnp.concatenate(
                [jnp.broadcast_to(lat_v[b, pl.ds(h, 1), :], (8, d_lat))
                 for b in range(n_batch)], axis=0,
            ).astype(jnp.bfloat16)
            ctx_v[0, h] = _dot(ctx_lat, wv_pair[i])
        pace_uv(j)

    pace_b = pacer(at_b, _B_ROUNDS, 2 * n_bh)

    @pl.loop(0, n_groups)
    def _(g):
        slot = g % 2
        _wait_filled(k_v.at[slot], block_sem(first_kv + 2 * g))

        @pl.loop(0, _STREAMS)
        def _(i):
            q = qb_v[i * n_groups + g].astype(jnp.bfloat16)
            s = _dot(q, k_v[slot, i], _NT) * scale
            p = jnp.exp(s - jnp.max(s, axis=-1, keepdims=True))
            p_v[i] = p / jnp.sum(p, axis=-1, keepdims=True)
            pace_b(2 * g * _STREAMS + i)

        _wait_filled(v_v.at[slot], block_sem(first_kv + 2 * g + 1))

        @pl.loop(0, _STREAMS)
        def _(i):
            bh = i * n_groups + g
            ctx = _dot(p_v[i].astype(jnp.bfloat16), v_v[slot, i])
            ctx_v[1, bh % n_heads, _aligned((bh // n_heads) * 8, 8), :] = ctx
            pace_b((2 * g + 1) * _STREAMS + i)

    def project(acc, which, heads, streams=range(half)):
        wo_v = (woa_v, wob_v)[which]
        for i in heads:
            for s in streams:
                ctx = ctx_v[which, s * heads_per_stream + i].astype(jnp.bfloat16)
                acc = acc + _dot(ctx, wo_v[s, i])
        return acc

    def project_first(which, n):
        return jax.lax.fori_loop(
            0, n // 2,
            lambda i, acc: project(acc, which, (2 * i, 2 * i + 1)),
            jnp.zeros((16, d_model), jnp.float32),
        )

    _wait_filled(woa_v.at[:, 0:6], wo_sem(0))
    _wait_filled(wob_v.at[:, 0:4], wo_sem(0))
    out_a = project_first(0, 6)
    out_b = project_first(1, 4)
    _wait_filled(wob_v.at[:, 4:6], wo_sem(1))
    out_b = project(out_b, 1, (4, 5))
    _wait_filled(woa_v.at[:, 6:8], wo_sem(2))
    out_a = project(out_a, 0, (6, 7))
    _wait_filled(wob_v.at[:, 6], wo_sem(3))
    out_b = project(out_b, 1, (6,))
    for i, (s, n) in enumerate(zip(tail_first, _TAIL)):
        _wait_filled(wob_v.at[s:s + n, 7], wo_sem(_BLOCK_SEMS + i))
        out_b = project(out_b, 1, (7,), range(s, s + n))

    out = jnp.concatenate([out_a, out_b], axis=1)
    out = jnp.concatenate([out[8 * b:8 * b + 1] for b in range(n_batch)], axis=0)
    out_ref[...] = out.astype(out_ref.dtype)


@jax.jit
def pallas_concat_heads__compressed_kv_cla__gqa_block_cached__decode_kernel(
    A_x: jax.Array,
    A_c_kv: jax.Array,
    A_w_q: jax.Array,
    A_w_uk: jax.Array,
    A_w_uv: jax.Array,
    A_w_o: jax.Array,
    B_x: jax.Array,
    B_k_cache: jax.Array,
    B_v_cache: jax.Array,
    B_wq: jax.Array,
    B_wo: jax.Array,
):
    n_batch, n_q, d_model = A_x.shape
    _, n_heads, n_kv, d_head = B_k_cache.shape
    d_lat = A_c_kv.shape[-1]
    assert n_batch == 2 and n_q == 1 and B_x.shape == A_x.shape
    assert A_c_kv.shape[1] == n_kv and A_w_q.shape[1:] == (n_heads, d_head)
    assert B_wq.shape == (d_model, n_heads * d_head)

    wo_shape = (_STREAMS // 2, 2 * n_heads // _STREAMS, d_head, d_model)
    xa = A_x.reshape(n_batch, d_model)
    xb = B_x.reshape(n_batch, d_model)
    ckv = A_c_kv.reshape(-1, d_lat)
    wqa = A_w_q.reshape(-1, d_head)
    wuk = A_w_uk.reshape(-1, d_head)
    wuv = A_w_uv.reshape(-1, d_head)
    woa = A_w_o.reshape(wo_shape)
    wob = B_wo.reshape(wo_shape)
    k = B_k_cache.reshape(_STREAMS, -1, n_kv, d_head)
    v = B_v_cache.reshape(_STREAMS, -1, n_kv, d_head)

    def vmem_like(x):
        return pltpu.VMEM(x.shape, x.dtype)

    def vmem_words(x):
        return pltpu.VMEM((x.shape[0] // 2, x.shape[1]), jnp.uint32)

    out = pl.pallas_call(
        _kernel,
        in_specs=[pl.BlockSpec(memory_space=pltpu.HBM)] * 11,
        out_specs=pl.BlockSpec(memory_space=pltpu.VMEM),
        out_shape=jax.ShapeDtypeStruct((n_batch, 2 * d_model), A_x.dtype),
        scratch_shapes=[
            vmem_like(xa),
            vmem_like(xb),
            vmem_like(ckv),
            vmem_words(wqa),
            vmem_words(wuk),
            vmem_words(wuv),
            vmem_like(B_wq),
            vmem_like(woa),
            vmem_like(wob),
            pltpu.VMEM((2, _STREAMS, n_kv, d_head), k.dtype),
            pltpu.VMEM((2, _STREAMS, n_kv, d_head), v.dtype),
            pltpu.VMEM((n_batch * n_heads, 8, d_head), jnp.float32),
            pltpu.VMEM((n_batch, n_heads, d_lat), jnp.float32),
            pltpu.VMEM((n_kv // _A_CHUNK, n_heads, _A_CHUNK), jnp.float32),
            pltpu.VMEM((_STREAMS, 8, n_kv), jnp.float32),
            pltpu.VMEM((2, n_heads, 16, d_head), jnp.float32),
            pltpu.SemaphoreType.DMA((_BLOCK_SEMS + len(_TAIL),)),
        ],
        compiler_params=pltpu.CompilerParams(
            vmem_limit_bytes=100 * 1024 * 1024,
            disable_bounds_checks=True,
        ),
    )(xa, ckv, wqa, wuk, wuv, woa, xb, k, v, B_wq, wob)
    return out.reshape(n_batch, n_q, 2 * d_model)
```

```python
import jax
import jax.numpy as jnp
import jax.experimental.pallas as pl
import jax.experimental.pallas.tpu as pltpu

_STREAMS = 8
_ROUNDS = 32
_BLOCK_SEMS = 4
_TAIL = (2, 1, 1)
_A_CHUNK = 512

_FILL_ROUNDS = 3
_LEAD_ROUNDS = 44
_WORDS_ROUNDS, _QA_ROUNDS, _QB_ROUNDS = 8, 50, 16
_ATT_ROUNDS, _UV_ROUNDS, _B_ROUNDS = 40, 20, 474

_NT = (((1,), (1,)), ((), ()))
_NN = (((1,), (0,)), ((), ()))


def _dot(a, b, dims=_NN):
    return jax.lax.dot_general(a, b, dims, preferred_element_type=jnp.float32)


def _rows_per_batch(x_ref):
    n = x_ref.shape[-1]
    x = x_ref[...].astype(jnp.float32)
    rows = [jnp.broadcast_to(x[b:b + 1], (8, n)) for b in range(2)]
    return jnp.concatenate(rows, axis=0).astype(jnp.bfloat16)


def _aligned(first, size):
    return pl.ds(pl.multiple_of(first, size), size)


def _to_words(w_ref, w32_ref, i, steps):
    n = w32_ref.shape[0] // steps
    w32_ref[_aligned(i * n, n), :] = pltpu.bitcast(
        w_ref[_aligned(i * 2 * n, 2 * n), :], jnp.uint32
    )


def _head_pair(w32_ref, j, n_pairs):
    w = w32_ref[pl.ds(j, w32_ref.shape[0] // n_pairs, stride=n_pairs), :]
    lo = pltpu.bitcast(w << 16, jnp.float32)
    hi = pltpu.bitcast(w & jnp.uint32(0xFFFF0000), jnp.float32)
    return lo.astype(jnp.bfloat16), hi.astype(jnp.bfloat16)


def _interleave(a, b):
    return [x for pair in zip(a, b, strict=True) for x in pair]


def _wait_filled(dst, sem):
    pltpu.make_async_copy(dst, dst, sem).wait()


def _kernel(
    xa_hbm, ckv_hbm, wqa_hbm, wuk_hbm, wuv_hbm, woa_hbm,
    xb_hbm, k_hbm, v_hbm, wqb_hbm, wob_hbm,
    out_ref,
    xa_v, xb_v, ckv_v, wqa_v, wuk_v, wuv_v, wqb_v, woa_v, wob_v, k_v, v_v,
    words0_v, words1_v, qb_v, lat_v, s_v, p_v, ctx_v,
    sems,
):
    _, n_groups, n_kv, d_head = k_hbm.shape
    n_batch, d_model = xa_hbm.shape
    n_bh = _STREAMS * n_groups
    n_heads = n_bh // n_batch
    n_pairs = n_heads // 2
    d_lat = ckv_hbm.shape[-1]
    n_chunks = n_kv // _A_CHUNK
    scale = d_head ** -0.5
    half = _STREAMS // 2
    heads_per_stream = n_heads // half

    first_kv = 3
    wo_block = first_kv + 2 * n_groups

    def block_sem(n):
        return sems.at[n % _BLOCK_SEMS]

    def start(pieces, threads=(0, 1) * half):
        for (src, dst, sem), thread in zip(pieces, threads, strict=True):
            pltpu.make_async_copy(src, dst, sem).start(priority=thread)

    def row_pieces(src, dst, sem, r, n_streams):
        n = src.shape[0] // (n_streams * _ROUNDS)
        rows = [_aligned((s * _ROUNDS + r) * n, n) for s in range(n_streams)]
        return [(src.at[x], dst.at[x], sem) for x in rows]

    def round_qa(r, **kwargs):
        start(_interleave(
            row_pieces(wqa_hbm, wqa_v, block_sem(0), r, half),
            row_pieces(wuk_hbm, wuk_v, block_sem(0), r, half),
        ), **kwargs)

    def round_qb(r):
        per_stream = wqb_hbm.shape[0] // half
        cols = _aligned((r % 2) * (wqb_hbm.shape[1] // 2), wqb_hbm.shape[1] // 2)
        rows = [_aligned(s * per_stream + (r // 2) * 8, 8) for s in range(half)]
        start(_interleave(
            [(wqb_hbm.at[x, cols], wqb_v.at[x, cols], block_sem(1)) for x in rows],
            row_pieces(wuv_hbm, wuv_v, block_sem(1), r, half),
        ))

    def round_ckv(r):
        start(row_pieces(ckv_hbm, ckv_v, block_sem(2), r, _STREAMS))

    def round_kv(r):
        block, r = r // _ROUNDS, r % _ROUNDS
        g = block // 2
        sem = block_sem(first_kv + block)
        rows = _aligned(r * (n_kv // _ROUNDS), n_kv // _ROUNDS)

        def cache(src, dst):
            start([
                (src.at[s, g, rows], dst.at[g % 2, s, rows], sem)
                for s in range(_STREAMS)
            ])

        pl.when(block % 2 == 0)(lambda: cache(k_hbm, k_v))
        pl.when(block % 2 == 1)(lambda: cache(v_hbm, v_v))

    per_head = _ROUNDS // heads_per_stream
    last = _ROUNDS - per_head
    tail_first = [sum(_TAIL[:i]) for i in range(len(_TAIL))]
    assert sum(_TAIL) == half == per_head and heads_per_stream == 8

    def wo_sem(i):
        if isinstance(i, int):
            return sems.at[i] if i >= _BLOCK_SEMS else block_sem(wo_block + i)
        return sems.at[jnp.where(i >= _BLOCK_SEMS, i, (wo_block + i) % _BLOCK_SEMS)]

    def round_wo(r):
        head = r // per_head
        n = d_head // per_head
        in_tail = r >= last
        tail_sem = _BLOCK_SEMS - 1 + sum(
            (r - last >= s).astype(jnp.int32) for s in tail_first
        )
        sem_a = wo_sem(jnp.where(head < 6, 0, 2))
        sem_b = wo_sem(jnp.where(
            head < 4, 0, jnp.where(head < 6, 1, jnp.where(in_tail, tail_sem, 3))
        ))
        pieces = []
        for s in range(half):
            at = (s, head, _aligned((r % per_head) * n, n))
            pieces.append((woa_hbm.at[at], woa_v.at[at], sem_a))
            at = (
                jnp.where(in_tail, r - last, s),
                head,
                _aligned(jnp.where(in_tail, s, r % per_head) * n, n),
            )
            pieces.append((wob_hbm.at[at], wob_v.at[at], sem_b))
        start(pieces)

    segments = []
    for n, fn in (
        (1, round_qa), (1, round_qb), (1, round_ckv),
        (2 * n_groups, round_kv), (1, round_wo),
    ):
        first = segments[-1][1] if segments else 0
        segments.append((first, first + n * _ROUNDS, fn))
    n_rounds = segments[-1][1]

    def issue(lo, hi, bounds):
        live = [s for s in segments if s[0] < bounds[1] and bounds[0] < s[1]]

        def one(r, carry):
            for first, end, fn in live:
                if len(live) == 1:
                    fn(r - first)
                else:
                    pl.when((r >= first) & (r < end))(
                        lambda first=first, fn=fn: fn(r - first)
                    )
            return carry

        jax.lax.fori_loop(lo, hi, one, 0)

    def pacer(first, n, steps):
        end = min(first + n, n_rounds)

        def pace(step):
            lo = first + step * n // steps
            hi = first + (step + 1) * n // steps
            issue(jnp.minimum(lo, end), jnp.minimum(hi, end), (first, end))

        return pace

    at_words = _LEAD_ROUNDS
    at_qa = at_words + _WORDS_ROUNDS
    at_qb = at_qa + _QA_ROUNDS
    at_att = at_qb + _QB_ROUNDS
    at_uv = at_att + _ATT_ROUNDS
    at_b = at_uv + _UV_ROUNDS
    waited = [at_words, at_qb, at_att] + [
        at_b + i * _STREAMS * _B_ROUNDS // (2 * n_bh)
        for i in range(2 * n_groups + 1)
    ]
    for n in range(wo_block):
        assert (n + 1) * _ROUNDS <= waited[n]
        assert waited[n + (n >= first_kv)] <= (n + _BLOCK_SEMS) * _ROUNDS
    for i, head in enumerate((0, 4, 6, 6)):
        taken_over = wo_block * _ROUNDS + head * per_head
        assert waited[wo_block + i - _BLOCK_SEMS] <= taken_over
    assert waited[-1] >= n_rounds

    @pl.loop(0, _FILL_ROUNDS)
    def _(r):
        round_qa(r, threads=(1,) * _STREAMS)

    x_copies = [
        pltpu.make_async_copy(xa_hbm, xa_v, block_sem(0)),
        pltpu.make_async_copy(xb_hbm, xb_v, block_sem(0)),
    ]
    for cp in x_copies:
        cp.start()
    issue(_FILL_ROUNDS, at_words, (_FILL_ROUNDS, at_words))

    for cp in x_copies:
        cp.wait()
    _wait_filled(wqa_v, block_sem(0))
    _wait_filled(wuk_v, block_sem(0))
    pace_words = pacer(at_words, _WORDS_ROUNDS, _WORDS_ROUNDS)

    @pl.loop(0, _WORDS_ROUNDS)
    def _(i):
        _to_words(wqa_v, words0_v, i, _WORDS_ROUNDS)
        _to_words(wuk_v, words1_v, i, _WORDS_ROUNDS)
        pace_words(i)

    xa = _rows_per_batch(xa_v)
    pace_qa = pacer(at_qa, _QA_ROUNDS, n_pairs)

    @pl.loop(0, n_pairs)
    def _(j):
        wq_pair = _head_pair(words0_v, j, n_pairs)
        wk_pair = _head_pair(words1_v, j, n_pairs)
        for i in range(2):
            q = _dot(xa, wq_pair[i]).astype(jnp.bfloat16)
            q_lat = _dot(q, wk_pair[i], _NT)
            for b in range(n_batch):
                lat_v[b, pl.ds(2 * j + i, 1), :] = q_lat[8 * b:8 * b + 1]
        pace_qa(j)

    _wait_filled(wqb_v, block_sem(1))
    _wait_filled(wuv_v, block_sem(1))
    xb = _rows_per_batch(xb_v)
    pace_qb = pacer(at_qb, _QB_ROUNDS, n_heads // 4)

    @pl.loop(0, n_heads // 4)
    def _(j):
        q = _dot(xb, wqb_v[:, _aligned(j * 4 * d_head, 4 * d_head)])
        for i in range(4):
            for b in range(n_batch):
                qb_v[b * n_heads + j * 4 + i] = q[
                    8 * b:8 * b + 8, i * d_head:(i + 1) * d_head
                ]
        _to_words(wuv_v, words0_v, j, n_heads // 4)
        pace_qb(j)

    _wait_filled(ckv_v, block_sem(2))
    pace_att = pacer(at_att, _ATT_ROUNDS, n_batch * n_chunks * 3)

    @pl.loop(0, n_batch)
    def _(b):
        q_lat = lat_v[b].astype(jnp.bfloat16)

        def keys(c):
            return ckv_v[_aligned(b * n_kv + c * _A_CHUNK, _A_CHUNK), :]

        def scores(c, m):
            s = _dot(q_lat, keys(c), _NT) * scale
            s_v[c] = s

            @pl.loop(0, 2)
            def _(i):
                pace_att(b * 3 * n_chunks + 2 * c + i)

            return jnp.maximum(m, jnp.max(s, axis=-1, keepdims=True))

        m = jax.lax.fori_loop(
            0, n_chunks, scores, jnp.full((n_heads, 1), -jnp.inf, jnp.float32)
        )

        def values(c, carry):
            l, acc = carry
            p = jnp.exp(s_v[c] - m)
            l = l + jnp.sum(p, axis=-1, keepdims=True)
            acc = acc + _dot(p.astype(jnp.bfloat16), keys(c))
            pace_att((b * 3 + 2) * n_chunks + c)
            return l, acc

        l, acc = jax.lax.fori_loop(
            0, n_chunks, values,
            (jnp.zeros((n_heads, 1), jnp.float32),
             jnp.zeros((n_heads, d_lat), jnp.float32)),
        )
        lat_v[b] = acc / l

    pace_uv = pacer(at_uv, _UV_ROUNDS, n_pairs)

    @pl.loop(0, n_pairs)
    def _(j):
        wv_pair = _head_pair(words0_v, j, n_pairs)
        for i in range(2):
            h = 2 * j + i
            ctx_lat = jnp.concatenate(
                [jnp.broadcast_to(lat_v[b, pl.ds(h, 1), :], (8, d_lat))
                 for b in range(n_batch)], axis=0,
            ).astype(jnp.bfloat16)
            ctx_v[0, h] = _dot(ctx_lat, wv_pair[i])
        pace_uv(j)

    pace_b = pacer(at_b, _B_ROUNDS, 2 * n_bh)

    @pl.loop(0, n_groups)
    def _(g):
        slot = g % 2
        _wait_filled(k_v.at[slot], block_sem(first_kv + 2 * g))

        @pl.loop(0, _STREAMS)
        def _(i):
            q = qb_v[i * n_groups + g].astype(jnp.bfloat16)
            s = _dot(q, k_v[slot, i], _NT) * scale
            p = jnp.exp(s - jnp.max(s, axis=-1, keepdims=True))
            p_v[i] = p / jnp.sum(p, axis=-1, keepdims=True)
            pace_b(2 * g * _STREAMS + i)

        _wait_filled(v_v.at[slot], block_sem(first_kv + 2 * g + 1))

        @pl.loop(0, _STREAMS)
        def _(i):
            bh = i * n_groups + g
            ctx = _dot(p_v[i].astype(jnp.bfloat16), v_v[slot, i])
            ctx_v[1, bh % n_heads, _aligned((bh // n_heads) * 8, 8), :] = ctx
            pace_b((2 * g + 1) * _STREAMS + i)

    def project(acc, which, heads, streams=range(half)):
        wo_v = (woa_v, wob_v)[which]
        for i in heads:
            for s in streams:
                ctx = ctx_v[which, s * heads_per_stream + i].astype(jnp.bfloat16)
                acc = acc + _dot(ctx, wo_v[s, i])
        return acc

    def project_first(which, n):
        return jax.lax.fori_loop(
            0, n // 2,
            lambda i, acc: project(acc, which, (2 * i, 2 * i + 1)),
            jnp.zeros((16, d_model), jnp.float32),
        )

    _wait_filled(woa_v.at[:, 0:6], wo_sem(0))
    _wait_filled(wob_v.at[:, 0:4], wo_sem(0))
    out_a = project_first(0, 6)
    out_b = project_first(1, 4)
    _wait_filled(wob_v.at[:, 4:6], wo_sem(1))
    out_b = project(out_b, 1, (4, 5))
    _wait_filled(woa_v.at[:, 6:8], wo_sem(2))
    out_a = project(out_a, 0, (6, 7))
    _wait_filled(wob_v.at[:, 6], wo_sem(3))
    out_b = project(out_b, 1, (6,))
    for i, (s, n) in enumerate(zip(tail_first, _TAIL)):
        _wait_filled(wob_v.at[s:s + n, 7], wo_sem(_BLOCK_SEMS + i))
        out_b = project(out_b, 1, (7,), range(s, s + n))

    out = jnp.concatenate([out_a, out_b], axis=1)
    out = jnp.concatenate([out[8 * b:8 * b + 1] for b in range(n_batch)], axis=0)
    out_ref[...] = out.astype(out_ref.dtype)


@jax.jit
def pallas_concat_heads__compressed_kv_cla__gqa_block_cached__decode_kernel(
    A_x: jax.Array,
    A_c_kv: jax.Array,
    A_w_q: jax.Array,
    A_w_uk: jax.Array,
    A_w_uv: jax.Array,
    A_w_o: jax.Array,
    B_x: jax.Array,
    B_k_cache: jax.Array,
    B_v_cache: jax.Array,
    B_wq: jax.Array,
    B_wo: jax.Array,
):
    n_batch, n_q, d_model = A_x.shape
    _, n_heads, n_kv, d_head = B_k_cache.shape
    d_lat = A_c_kv.shape[-1]
    assert n_batch == 2 and n_q == 1 and B_x.shape == A_x.shape
    assert A_c_kv.shape[1] == n_kv and A_w_q.shape[1:] == (n_heads, d_head)
    assert B_wq.shape == (d_model, n_heads * d_head)

    wo_shape = (_STREAMS // 2, 2 * n_heads // _STREAMS, d_head, d_model)
    xa = A_x.reshape(n_batch, d_model)
    xb = B_x.reshape(n_batch, d_model)
    ckv = A_c_kv.reshape(-1, d_lat)
    wqa = A_w_q.reshape(-1, d_head)
    wuk = A_w_uk.reshape(-1, d_head)
    wuv = A_w_uv.reshape(-1, d_head)
    woa = A_w_o.reshape(wo_shape)
    wob = B_wo.reshape(wo_shape)
    k = B_k_cache.reshape(_STREAMS, -1, n_kv, d_head)
    v = B_v_cache.reshape(_STREAMS, -1, n_kv, d_head)

    def vmem_like(x):
        return pltpu.VMEM(x.shape, x.dtype)

    def vmem_words(x):
        return pltpu.VMEM((x.shape[0] // 2, x.shape[1]), jnp.uint32)

    out = pl.pallas_call(
        _kernel,
        in_specs=[pl.BlockSpec(memory_space=pltpu.HBM)] * 11,
        out_specs=pl.BlockSpec(memory_space=pltpu.VMEM),
        out_shape=jax.ShapeDtypeStruct((n_batch, 2 * d_model), A_x.dtype),
        scratch_shapes=[
            vmem_like(xa),
            vmem_like(xb),
            vmem_like(ckv),
            vmem_like(wqa),
            vmem_like(wuk),
            vmem_like(wuv),
            vmem_like(B_wq),
            vmem_like(woa),
            vmem_like(wob),
            pltpu.VMEM((2, _STREAMS, n_kv, d_head), k.dtype),
            pltpu.VMEM((2, _STREAMS, n_kv, d_head), v.dtype),
            vmem_words(wqa),
            vmem_words(wuk),
            pltpu.VMEM((n_batch * n_heads, 8, d_head), jnp.float32),
            pltpu.VMEM((n_batch, n_heads, d_lat), jnp.float32),
            pltpu.VMEM((n_kv // _A_CHUNK, n_heads, _A_CHUNK), jnp.float32),
            pltpu.VMEM((_STREAMS, 8, n_kv), jnp.float32),
            pltpu.VMEM((2, n_heads, 16, d_head), jnp.float32),
            pltpu.SemaphoreType.DMA((_BLOCK_SEMS + len(_TAIL),)),
        ],
        compiler_params=pltpu.CompilerParams(
            vmem_limit_bytes=100 * 1024 * 1024,
            disable_bounds_checks=True,
        ),
    )(xa, ckv, wqa, wuk, wuv, woa, xb, k, v, B_wq, wob)
    return out.reshape(n_batch, n_q, 2 * d_model)
```
